```python
import jax
import jax.numpy as jnp

def _softmax(x, axis=-1):
    return jax.nn.softmax(x, axis=axis)
def _gelu(x):
    return jax.nn.gelu(x, approximate=True)
def _silu(x):
    return jax.nn.silu(x)
def _sigmoid(x):
    return jax.nn.sigmoid(x)
def _layernorm(x, axis=-1, eps=1e-5):
    m = jnp.mean(x, axis=axis, keepdims=True)
    v = jnp.var(x, axis=axis, keepdims=True)
    return (x - m) / jnp.sqrt(v + eps)
def _scatter_add(tgt, idx, src, axis=0):
    return tgt.at[idx].add(src)
def _segment_sum(src, seg, n):
    return jax.ops.segment_sum(src, seg, n)
class _Rng:
    def __init__(self, key):
        self._k = key
    def _next(self):
        self._k, sub = jax.random.split(self._k)
        return sub
    def normal(self, shape):
        return jax.random.normal(self._next(), shape, dtype=jnp.bfloat16)
    def randint(self, lo, hi, shape):
        return jax.random.randint(self._next(), shape, lo, hi, dtype=jnp.int32)
    def uniform(self, shape, lo=0.0, hi=1.0):
        return jax.random.uniform(self._next(), shape, jnp.bfloat16, lo, hi)
    def permutation(self, n):
        return jax.random.permutation(self._next(), n)


kernel_name = 'gated_mix__sliding_block_cached__mixer_s_mlp__decode'

def setup_inputs():
    _rng = _Rng(jax.random.key(int.from_bytes(__import__("os").urandom(4), "little")))
    _w = (lambda a: (lambda t: t.astype(jnp.bfloat16) if jnp.issubdtype(t.dtype, jnp.floating) else t)(jnp.asarray(a)))
    def _A_setup():
        B, Sq, D = 1, 1, 576
        Hq, Hkv, Sk, Dh = 32, 16, 65536, 128
        assert Hq % Hkv == 0, (Hq, Hkv)
        return {
            "x": _w((lambda *s: _rng.normal(s) * 0.05)(B, Sq, D)),
            "k_cache": _w((lambda *s: _rng.normal(s) * 0.05)(B, Hkv, Sk, Dh)),
            "v_cache": _w((lambda *s: _rng.normal(s) * 0.05)(B, Hkv, Sk, Dh)),
            "wq": _w((lambda *s: _rng.normal(s) * 0.05)(D, Hq * Dh) * (D ** -0.5)),
            "wo": _w((lambda *s: _rng.normal(s) * 0.05)(Hq * Dh, D) * ((Hq * Dh) ** -0.5)),
        }
    _A_in = _A_setup()

    def _B_setup():
        B, S, D, F = 1, 1, 576, 4608
        return {
            "x":  _w((lambda *s: _rng.normal(s) * 0.05)(B, S, D)),
            "w1": _w((lambda *s: _rng.normal(s) * 0.05)(D, D) * (D ** -0.5)),
            "w2": _w((lambda *s: _rng.normal(s) * 0.05)(D, D) * (D ** -0.5)),
            "w3": _w((lambda *s: _rng.normal(s) * 0.05)(D, F) * (D ** -0.5)),
            "w4": _w((lambda *s: _rng.normal(s) * 0.05)(F, D) * (F ** -0.5)),
        }
    _B_in = _B_setup()

    return {
        "A_x": _A_in["x"],
        "A_k_cache": _A_in["k_cache"],
        "A_v_cache": _A_in["v_cache"],
        "A_wq": _A_in["wq"],
        "A_wo": _A_in["wo"],
        "B_x": _B_in["x"],
        "B_w1": _B_in["w1"],
        "B_w2": _B_in["w2"],
        "B_w3": _B_in["w3"],
        "B_w4": _B_in["w4"],
        "gate_w": _w((lambda *s: _rng.normal(s) * 0.05)(576)),
    }

def reference(A_x, A_k_cache, A_v_cache, A_wq, A_wo, B_x, B_w1, B_w2, B_w3, B_w4, gate_w):
    def _A_ref(x, k_cache, v_cache, wq, wo):
        B, Sq, D = x.shape
        Hq, Dh = 32, 128
        Hkv, Sk = k_cache.shape[1], k_cache.shape[2]
        W = min(4096, max(256, Sk // 4))
        rep = Hq // Hkv
        q = (lambda x, *d: x.transpose(*d))((x @ wq).reshape(B, Sq, Hq, Dh), 0, 2, 1, 3)
        k = jnp.repeat(k_cache[:, :, Sk - W:, :], rep, axis=1)
        v = jnp.repeat(v_cache[:, :, Sk - W:, :], rep, axis=1)
        scores = jnp.einsum("bhqd,bhkd->bhqk", q, k) * (Dh ** -0.5)
        p = _softmax(scores, axis=-1)
        o = jnp.einsum("bhqk,bhkd->bhqd", p, v)
        return (lambda x, *d: x.transpose(*d))(o, 0, 2, 1, 3).reshape(B, Sq, Hq * Dh) @ wo

    def _B_ref(x, w1, w2, w3, w4):
        B, S, D = x.shape
        h = _gelu(_layernorm(x, axis=-1) @ w1)
        c = D // 4
        g0 = jnp.pad(h[:, :, 0*c:1*c], ((0, 0), (1, 0), (0, 0)))[:, :S, :]
        g1 = jnp.pad(h[:, :, 1*c:2*c], ((0, 0), (0, 1), (0, 0)))[:, 1:, :]
        g2 = jnp.pad(h[:, :, 2*c:3*c], ((0, 0), (2, 0), (0, 0)))[:, :S, :]
        g3 = jnp.pad(h[:, :, 3*c:   ], ((0, 0), (0, 2), (0, 0)))[:, 2:, :]
        hs = jnp.concatenate([g0, g1, g2, g3], axis=-1) @ w2
        x1 = x + hs
        h2 = _gelu(_layernorm(x1, axis=-1) @ w3) @ w4
        return x1 + h2

    x = A_x
    g = _sigmoid((x * gate_w).sum(-1, keepdims=True))
    a = _A_ref(x, A_k_cache, A_v_cache, A_wq, A_wo)
    b = _B_ref(x, B_w1, B_w2, B_w3, B_w4)
    return g * a + (1 - g) * b
```

```python
import jax
import jax.numpy as jnp
from jax import lax
import jax.experimental.pallas as pl
import jax.experimental.pallas.tpu as pltpu

F32, BF16 = jnp.float32, jnp.bfloat16
HQ, DH = 32, 128
NT = (((1,), (1,)), ((), ()))


def _gelu(x):
    return 0.5 * x * (1.0 + jnp.tanh(0.7978845608028654 * (x + 0.044715 * (x * x * x))))


@jax.jit
def pallas_gated_mix__sliding_block_cached__mixer_s_mlp__decode_kernel(
    A_x, A_k_cache, A_v_cache, A_wq, A_wo, B_x, B_w1, B_w2, B_w3, B_w4, gate_w,
):
    D = A_x.shape[-1]
    HKV, SK = A_k_cache.shape[1], A_k_cache.shape[2]
    F = B_w3.shape[1]
    W = min(4096, max(256, SK // 4))

    def kernel(x_ref, gw_ref, k, v, wq_h, wo_h, w3_h, w4_h, o_ref,
               kb, vb, wqb, wob, w3b, w4b, q_s, o_s, sems):
        c_wq = pltpu.make_async_copy(wq_h, wqb, sems.at[0])
        c_w3 = pltpu.make_async_copy(w3_h, w3b, sems.at[1])
        c_wo = pltpu.make_async_copy(wo_h, wob, sems.at[2])
        c_w4 = pltpu.make_async_copy(w4_h, w4b, sems.at[3])
        ck = lambda h: pltpu.make_async_copy(k.at[0, h, pl.ds(SK - W, W), :], kb.at[h], sems.at[4 + h])
        cv = lambda h: pltpu.make_async_copy(v.at[0, h, pl.ds(SK - W, W), :], vb.at[h], sems.at[4 + HKV + h])
        c_wq.start()
        c_w3.start(priority=1)
        x = x_ref[0].astype(F32)
        x8 = jnp.broadcast_to(x, (8, D))
        c_wq.wait()
        for h in range(2):
            ck(h).start()
            cv(h).start(priority=1)
        q = jnp.dot(x8.astype(BF16), wqb[...], preferred_element_type=F32)
        row = lax.broadcasted_iota(jnp.int32, (8, DH), 0)
        for h in range(HKV):
            q0 = q[:, (2 * h) * DH:(2 * h + 1) * DH]
            q1 = q[:, (2 * h + 1) * DH:(2 * h + 2) * DH]
            q_s[h] = jnp.where(row == 1, q1, q0)
        c_w3.wait()
        xc = x8 - jnp.mean(x8, axis=-1, keepdims=True)
        ln = xc / jnp.sqrt(jnp.mean(xc * xc, axis=-1, keepdims=True) + 1e-5)
        hmid = _gelu(jnp.dot(ln.astype(BF16), w3b[...], preferred_element_type=F32)).astype(BF16)

        def head(h, _):
            @pl.when(h + 2 < HKV)
            def _():
                ck(h + 2).start()
                cv(h + 2).start(priority=1)

            @pl.when(h == HKV - 2)
            def _():
                c_wo.start()
                c_w4.start(priority=1)

            ck(h).wait()
            s = lax.dot_general(q_s[h].astype(BF16), kb[h], NT, preferred_element_type=F32) * (DH ** -0.5)
            e = jnp.exp(s - jnp.max(s, axis=-1, keepdims=True))
            p = e / jnp.sum(e, axis=-1, keepdims=True)
            cv(h).wait()
            o_s[h] = jnp.dot(p.astype(BF16), vb[h], preferred_element_type=F32)
            return 0

        lax.fori_loop(0, HKV, head, 0)

        o = jnp.concatenate([o_s[h][j:j + 1, :] for h in range(HKV) for j in range(2)], axis=1)
        o8 = jnp.broadcast_to(o, (8, HQ * DH)).astype(BF16)
        c_wo.wait()
        a = lax.dot_general(o8, wob[...], NT, preferred_element_type=F32)
        c_w4.wait()
        b = x8 + lax.dot_general(hmid, w4b[...], NT, preferred_element_type=F32)
        g = jax.nn.sigmoid(jnp.sum(x * gw_ref[...].astype(F32).reshape(1, D), axis=-1, keepdims=True))
        o_ref[0] = (g * a[0:1] + (1.0 - g) * b[0:1]).astype(o_ref.dtype)

    hbm = pl.BlockSpec(memory_space=pl.ANY)
    vmem = pl.BlockSpec(memory_space=pltpu.VMEM)
    return pl.pallas_call(
        kernel,
        out_shape=jax.ShapeDtypeStruct(A_x.shape, A_x.dtype),
        in_specs=[vmem, vmem] + [hbm] * 6,
        out_specs=vmem,
        scratch_shapes=[
            pltpu.VMEM((HKV, W, DH), BF16), pltpu.VMEM((HKV, W, DH), BF16),
            pltpu.VMEM((D, HQ * DH), BF16), pltpu.VMEM((D, HQ * DH), BF16),
            pltpu.VMEM((D, F), BF16), pltpu.VMEM((D, F), BF16),
            pltpu.VMEM((HKV, 8, DH), F32), pltpu.VMEM((HKV, 8, DH), F32),
            pltpu.SemaphoreType.DMA((4 + 2 * HKV,)),
        ],
        compiler_params=pltpu.CompilerParams(vmem_limit_bytes=100 * 1024 * 1024),
    )(A_x, gate_w, A_k_cache, A_v_cache, A_wq, A_wo.T, B_w3, B_w4.T)
```

```python
import functools

import jax
import jax.numpy as jnp
from jax import lax
import jax.experimental.pallas as pl
import jax.experimental.pallas.tpu as pltpu

F32, BF16 = jnp.float32, jnp.bfloat16
HQ, DH = 32, 128
LANES, SUBLANES = 128, 8
CONTRACT_LAST = (((1,), (1,)), ((), ()))

GROUP = 8
COPY_HEADS = 2
COPY_ROWS = 64
STREAMS = 4
V_LAG = 3
TAIL_BURSTS = (32, 36) + (18,) * V_LAG + (24,) * (GROUP - 1 - V_LAG) + (12,) * V_LAG


def _gelu(x):
    return 0.5 * x * (1.0 + jnp.tanh(0.7978845608028654 * (x + 0.044715 * (x * x * x))))


def _interleave(*streams):
    keyed = [((i + 0.5) / len(s), k, item)
             for k, s in enumerate(streams) for i, item in enumerate(s)]
    keyed.sort(key=lambda t: t[:2])
    return [t[2] for t in keyed]


def _row_copies(src, dst, row0, row1, sem):
    half = src.shape[1] // 2
    return [(src, dst, r, c, half, sem)
            for r in range(row0, row1, SUBLANES) for c in (0, half)]


def _kernel(x_hbm, gate_hbm, k_hbm, v_hbm, wq_hbm, wo_hbm, w3_hbm, w4_hbm, out_ref,
            x_buf, gate_buf, k_buf, v_buf, wq_buf, wo_buf, w3_buf, w4_buf,
            q_buf, p_buf, l_buf, o_buf, h_buf, sems):
    hkv, window, _ = k_buf.shape
    first_row = k_hbm.shape[2] - window
    d = wq_buf.shape[0]
    step_rows = window // GROUP
    full_slabs = d // LANES
    sem_x, sem_head, sem_kv = 0, 1, 2
    sem_wo = sem_kv + 2 * (hkv // GROUP)
    sem_w4 = sem_wo + 1

    def start_rows(src, dst, row, col, ncols, sem, priority):
        idx = (pl.ds(row, SUBLANES), pl.ds(col, ncols))
        pltpu.make_async_copy(src.at[idx], dst.at[idx], sems.at[sem]).start(priority=priority)

    def wait(filled, sem):
        pltpu.make_async_copy(filled, filled, sems.at[sem]).wait()

    def start_kv(step):
        group = step // GROUP
        row0 = (step % GROUP) * step_rows
        if not isinstance(row0, int):
            row0 = pl.multiple_of(row0, step_rows)
        for r in range(0, step_rows, COPY_ROWS):
            for dh in range(0, GROUP, COPY_HEADS):
                heads = pl.ds(group * GROUP + dh, COPY_HEADS)
                for queue, (src, dst) in enumerate(((k_hbm, k_buf), (v_hbm, v_buf))):
                    pltpu.make_async_copy(
                        src.at[0, heads, pl.ds(first_row + row0 + r, COPY_ROWS), :],
                        dst.at[heads, pl.ds(row0 + r, COPY_ROWS), :],
                        sems.at[sem_kv + 2 * group + queue]).start(priority=queue)

    stream_rows = d // STREAMS
    head_copies = _interleave(*[
        _row_copies(src, dst, s * stream_rows, s * stream_rows + SUBLANES, sem_head)
        for s in range(STREAMS) for src, dst in ((wq_hbm, wq_buf), (w3_hbm, w3_buf))])

    def start_head(i, carry):
        row = pl.multiple_of(i * SUBLANES, SUBLANES)
        for j, (src, dst, r, c, ncols, sem) in enumerate(head_copies):
            start_rows(src, dst, row + r, c, ncols, sem, j % 2)
        return carry

    early = _interleave(
        *[_row_copies(wo_hbm, wo_buf, s * stream_rows, (s + 1) * stream_rows, sem_wo)
          for s in range(STREAMS)],
        _row_copies(w4_hbm, w4_buf, 0, LANES, sem_w4))
    for j in range(1, full_slabs):
        r = j * LANES
        early += _interleave(
            _row_copies(w4_hbm, w4_buf, r, r + LANES // 2, sem_w4 + j),
            _row_copies(w4_hbm, w4_buf, r + LANES // 2, r + LANES, sem_w4 + j))
    r, mid = full_slabs * LANES, (full_slabs * LANES + d) // 2
    late = _interleave(_row_copies(w4_hbm, w4_buf, r, mid, sem_w4 + full_slabs),
                       _row_copies(w4_hbm, w4_buf, mid, d, sem_w4 + full_slabs))
    paired = len(early) - len(late)
    tail_copies = [c + (i % 2,) for i, c in enumerate(early[:paired])]
    for c0, c1 in zip(early[paired:], late):
        tail_copies += [c0 + (0,), c1 + (1,)]

    def start_tail(lo, hi):
        for c in tail_copies[lo:hi]:
            start_rows(*c)

    x_copy = pltpu.make_async_copy(x_hbm, x_buf, sems.at[sem_x])
    gate_copy = pltpu.make_async_copy(gate_hbm, gate_buf, sems.at[sem_x])
    x_copy.start()
    gate_copy.start(priority=1)
    lax.fori_loop(0, stream_rows // SUBLANES, start_head, 0)
    x_copy.wait()
    gate_copy.wait()
    x = x_buf[0].astype(F32)
    x8 = jnp.broadcast_to(x, (SUBLANES, d))
    gate = jax.nn.sigmoid(
        jnp.sum(x * gate_buf[...].astype(F32).reshape(1, d), axis=-1, keepdims=True))

    start_kv(0)
    start_kv(1)
    wait(wq_buf, sem_head)
    wait(w3_buf, sem_head)
    q = jnp.dot(x8.astype(BF16), wq_buf[...], preferred_element_type=F32)
    second = lax.broadcasted_iota(jnp.int32, (SUBLANES, DH), 0) == 1
    for h in range(hkv):
        q_buf[h] = jnp.where(second, q[:, (2 * h + 1) * DH:(2 * h + 2) * DH],
                             q[:, 2 * h * DH:(2 * h + 1) * DH])

    start_kv(2)
    centered = x8 - jnp.mean(x8, axis=-1, keepdims=True)
    normed = centered / jnp.sqrt(jnp.mean(centered * centered, axis=-1, keepdims=True) + 1e-5)
    h_buf[...] = _gelu(jnp.dot(normed.astype(BF16), w3_buf[...], preferred_element_type=F32))

    def fill(step, carry):
        start_kv(step)
        return carry

    lax.fori_loop(3, GROUP + 1, fill, 0)

    last_group = hkv - GROUP
    kv_bursts = last_group - 1

    def head_step(h, carry):
        @pl.when(h < kv_bursts)
        def _():
            start_kv(h + GROUP + 1)

        lo = 0
        for i, count in enumerate(TAIL_BURSTS):
            pl.when(h == kv_bursts + i)(functools.partial(start_tail, lo, lo + count))
            lo += count

        @pl.when(h < hkv)
        def _():
            @pl.when(h % GROUP == 0)
            def _():
                wait(k_buf.at[pl.ds(h, GROUP)], sem_kv + 2 * (h // GROUP))

            s = lax.dot_general(q_buf[h].astype(BF16), k_buf[h], CONTRACT_LAST,
                                preferred_element_type=F32) * (DH ** -0.5)
            e = jnp.exp(s - jnp.max(s, axis=-1, keepdims=True))
            p_buf[h] = e
            l_buf[h] = jnp.broadcast_to(jnp.sum(e, axis=-1, keepdims=True), (SUBLANES, DH))

        @pl.when((h < last_group) | (h >= last_group + V_LAG))
        def _():
            hv = jnp.where(h < last_group, h, h - V_LAG)

            @pl.when(hv % GROUP == 0)
            def _():
                wait(v_buf.at[pl.ds(hv, GROUP)], sem_kv + 2 * (hv // GROUP) + 1)

            o_buf[hv] = jnp.dot(p_buf[hv].astype(BF16), v_buf[hv],
                                preferred_element_type=F32) / l_buf[hv]

        return carry

    lax.fori_loop(0, hkv + V_LAG, head_step, 0)
    start_tail(sum(TAIL_BURSTS), len(tail_copies))

    o = jnp.concatenate([o_buf[h, j:j + 1, :] for h in range(hkv) for j in range(2)], axis=1)
    o8 = jnp.broadcast_to(o, (SUBLANES, HQ * DH)).astype(BF16)
    wait(wo_buf, sem_wo)
    attn = lax.dot_general(o8, wo_buf[...], CONTRACT_LAST, preferred_element_type=F32)
    base = gate * attn[0:1] + (1.0 - gate) * x
    hidden = h_buf[...].astype(BF16)
    for j, c in enumerate(range(0, d, LANES)):
        n = min(LANES, d - c)
        slab = w4_buf.at[pl.ds(c, n)]
        wait(slab, sem_w4 + j)
        mlp = lax.dot_general(hidden, slab[...], CONTRACT_LAST, preferred_element_type=F32)
        out_ref[0, :, c:c + n] = (
            base[:, c:c + n] + (1.0 - gate) * mlp[0:1]).astype(out_ref.dtype)


@jax.jit
def pallas_gated_mix__sliding_block_cached__mixer_s_mlp__decode_kernel(
    A_x: jax.Array,
    A_k_cache: jax.Array,
    A_v_cache: jax.Array,
    A_wq: jax.Array,
    A_wo: jax.Array,
    B_x: jax.Array,
    B_w1: jax.Array,
    B_w2: jax.Array,
    B_w3: jax.Array,
    B_w4: jax.Array,
    gate_w: jax.Array,
):
    del B_x, B_w1, B_w2
    batch, seq, d = A_x.shape
    assert (batch, seq) == (1, 1)
    _, hkv, sk, _ = A_k_cache.shape
    f = B_w3.shape[1]
    window = min(4096, max(256, sk // 4))
    num_sems = 2 + 2 * (hkv // GROUP) + 1 + pl.cdiv(d, LANES)

    return pl.pallas_call(
        _kernel,
        out_shape=jax.ShapeDtypeStruct(A_x.shape, A_x.dtype),
        in_specs=[pl.BlockSpec(memory_space=pl.ANY)] * 8,
        out_specs=pl.BlockSpec(memory_space=pltpu.VMEM),
        scratch_shapes=[
            pltpu.VMEM(A_x.shape, A_x.dtype),
            pltpu.VMEM(gate_w.shape, gate_w.dtype),
            pltpu.VMEM((hkv, window, DH), BF16),
            pltpu.VMEM((hkv, window, DH), BF16),
            pltpu.VMEM((d, HQ * DH), BF16),
            pltpu.VMEM((d, HQ * DH), BF16),
            pltpu.VMEM((d, f), BF16),
            pltpu.VMEM((d, f), BF16),
            pltpu.VMEM((hkv, SUBLANES, DH), F32),
            pltpu.VMEM((hkv, SUBLANES, window), F32),
            pltpu.VMEM((hkv, SUBLANES, DH), F32),
            pltpu.VMEM((hkv, SUBLANES, DH), F32),
            pltpu.VMEM((SUBLANES, f), F32),
            pltpu.SemaphoreType.DMA((num_sems,)),
        ],
        compiler_params=pltpu.CompilerParams(
            vmem_limit_bytes=100 * 1024 * 1024,
            disable_semaphore_checks=True,
        ),
    )(A_x, gate_w, A_k_cache, A_v_cache, A_wq, A_wo.T, B_w3, B_w4.T)
```

```python
import functools

import jax
import jax.numpy as jnp
from jax import lax
import jax.experimental.pallas as pl
import jax.experimental.pallas.tpu as pltpu

F32, BF16 = jnp.float32, jnp.bfloat16
HQ, DH = 32, 128
LANES, SUBLANES = 128, 8
CONTRACT_LAST = (((1,), (1,)), ((), ()))

GROUP = 8
COPY_HEADS = 2
COPY_ROWS = 64
STEP_HEADS = 2
STREAMS = 3
FIRST_BURST = 84
STEP_BURST = 42
LAST_PARTS = 2
QUEUE0_LEAD = 8


def _gelu(x):
    return 0.5 * x * (1.0 + jnp.tanh(0.7978845608028654 * (x + 0.044715 * (x * x * x))))


def _interleave(*streams):
    keyed = [((i + 0.5) / len(s), k, item)
             for k, s in enumerate(streams) for i, item in enumerate(s)]
    keyed.sort(key=lambda t: t[:2])
    return [t[2] for t in keyed]


def _slab_copies(src, dst, sem, row0, row1, col0=None, dst_row=0):
    if col0 is None:
        half = src.shape[1] // 2
        parts = ((0, 0, half), (half, half, half))
    else:
        parts = ((col0, 0, dst.shape[1]),)
    return [(src, dst, r, src_col, r - dst_row, dst_col, cols, sem)
            for r in range(row0, row1, SUBLANES) for src_col, dst_col, cols in parts]


def _kernel(x_hbm, gate_hbm, k_hbm, v_hbm, wq_hbm, wo_hbm, w3_hbm, w4_hbm, out_ref,
            x_buf, gate_buf, k_buf, v_buf, wq_buf, wo_buf, w3_buf, w4_buf,
            q_buf, o_buf, h_buf, sems, *last_bufs):
    hkv, window, _ = k_buf.shape
    first_row = k_hbm.shape[2] - window
    d = wq_buf.shape[0]
    step_rows = window // GROUP
    stream_rows = d // STREAMS
    last_row = w4_buf.shape[0]
    full_slabs = last_row // LANES
    sem_x, sem_wq, sem_w3, sem_wo, sem_kv = range(5)
    sem_w4 = sem_kv + hkv // GROUP
    sem_last = sem_w4 + full_slabs

    def start_slab(src, dst, src_row, src_col, dst_row, dst_col, cols, sem, queue):
        pltpu.make_async_copy(
            src.at[pl.ds(src_row, SUBLANES), pl.ds(src_col, cols)],
            dst.at[pl.ds(dst_row, SUBLANES), pl.ds(dst_col, cols)],
            sems.at[sem]).start(priority=queue)

    def wait(filled, sem):
        pltpu.make_async_copy(filled, filled, sems.at[sem]).wait()

    def start_kv(step):
        group = step // GROUP
        row0 = (step % GROUP) * step_rows
        if not isinstance(row0, int):
            row0 = pl.multiple_of(row0, step_rows)
        for r in range(0, step_rows, COPY_ROWS):
            for dh in range(0, GROUP, COPY_HEADS):
                heads = pl.ds(group * GROUP + dh, COPY_HEADS)
                for queue, (src, dst) in enumerate(((k_hbm, k_buf), (v_hbm, v_buf))):
                    pltpu.make_async_copy(
                        src.at[0, heads, pl.ds(first_row + row0 + r, COPY_ROWS), :],
                        dst.at[heads, pl.ds(row0 + r, COPY_ROWS), :],
                        sems.at[sem_kv + group]).start(priority=queue)

    def wait_kv(group):
        for buf in (k_buf, v_buf):
            wait(buf.at[pl.ds(group * GROUP, GROUP)], sem_kv + group)

    head_copies = _interleave(*[
        _slab_copies(src, dst, sem, s * stream_rows, s * stream_rows + SUBLANES)
        for s in range(STREAMS)
        for src, dst, sem in ((wq_hbm, wq_buf, sem_wq), (w3_hbm, w3_buf, sem_w3))])

    def start_head(i, carry):
        row = pl.multiple_of(i * SUBLANES, SUBLANES)
        for j, (src, dst, src_row, src_col, dst_row, *rest) in enumerate(head_copies):
            start_slab(src, dst, row + src_row, src_col, row + dst_row, *rest, j % 2)
        return carry

    early = _interleave(
        *[_slab_copies(wo_hbm, wo_buf, sem_wo, s * stream_rows, (s + 1) * stream_rows)
          for s in range(STREAMS)],
        _slab_copies(w4_hbm, w4_buf, sem_w4, 0, LANES))
    for j in range(1, full_slabs):
        lo, mid, hi = j * LANES, j * LANES + LANES // 2, (j + 1) * LANES
        early += _interleave(_slab_copies(w4_hbm, w4_buf, sem_w4 + j, lo, mid),
                             _slab_copies(w4_hbm, w4_buf, sem_w4 + j, mid, hi))
    late, mid = [], (last_row + d) // 2
    for j, buf in enumerate(last_bufs):
        late += _interleave(*[
            _slab_copies(w4_hbm, buf, sem_last + j, lo, hi, j * buf.shape[1], last_row)
            for lo, hi in ((last_row, mid), (mid, d))])
    paired = len(late) - QUEUE0_LEAD
    tail_copies = [c + (i % 2,) for i, c in enumerate(early[:-paired])]
    for c0, c1 in zip(early[-paired:], late):
        tail_copies += [c0 + (0,), c1 + (1,)]
    tail_copies += [c + (1,) for c in late[paired:]]

    def start_tail(lo, hi):
        for c in tail_copies[lo:hi]:
            start_slab(*c)

    def attend(head0):
        weights = []
        for h in range(STEP_HEADS):
            s = lax.dot_general(q_buf[head0 + h].astype(BF16), k_buf[head0 + h],
                                CONTRACT_LAST, preferred_element_type=F32) * (DH ** -0.5)
            e = jnp.exp(s - jnp.max(s, axis=-1, keepdims=True))
            weights.append((e.astype(BF16), jnp.sum(e, axis=-1, keepdims=True)))
        for h, (e, total) in enumerate(weights):
            o_buf[head0 + h] = jnp.dot(e, v_buf[head0 + h], preferred_element_type=F32) / total

    x_copy = pltpu.make_async_copy(x_hbm, x_buf, sems.at[sem_x])
    gate_copy = pltpu.make_async_copy(gate_hbm, gate_buf, sems.at[sem_x])
    x_copy.start()
    gate_copy.start(priority=1)
    lax.fori_loop(0, stream_rows // SUBLANES, start_head, 0)
    x_copy.wait()
    gate_copy.wait()
    x = x_buf[0].astype(F32)
    x8 = jnp.broadcast_to(x, (SUBLANES, d))
    gate = jax.nn.sigmoid(
        jnp.sum(x * gate_buf[...].astype(F32).reshape(1, d), axis=-1, keepdims=True))

    start_kv(0)
    start_kv(1)
    wait(wq_buf, sem_wq)
    q = jnp.dot(x8.astype(BF16), wq_buf[...], preferred_element_type=F32)
    second = lax.broadcasted_iota(jnp.int32, (SUBLANES, DH), 0) == 1
    for h in range(hkv):
        q_buf[h] = jnp.where(second, q[:, (2 * h + 1) * DH:(2 * h + 2) * DH],
                             q[:, 2 * h * DH:(2 * h + 1) * DH])

    start_kv(2)
    wait(w3_buf, sem_w3)
    centered = x8 - jnp.mean(x8, axis=-1, keepdims=True)
    normed = centered / jnp.sqrt(jnp.mean(centered * centered, axis=-1, keepdims=True) + 1e-5)
    h_buf[...] = _gelu(jnp.dot(normed.astype(BF16), w3_buf[...], preferred_element_type=F32))

    def fill(step, carry):
        start_kv(step)
        return carry

    lax.fori_loop(3, GROUP + 2, fill, 0)
    wait_kv(0)
    steps = GROUP // STEP_HEADS

    def attend_first_group(i, carry):
        attend(i * STEP_HEADS)
        for j in range(STEP_HEADS):
            step = GROUP + 2 + i * STEP_HEADS + j
            pl.when(step < hkv)(functools.partial(start_kv, step))
        return carry

    lax.fori_loop(0, steps, attend_first_group, 0)
    start_tail(0, FIRST_BURST)
    wait_kv(1)

    def attend_second_group(i, carry):
        attend(GROUP + i * STEP_HEADS)
        for j in range(steps):
            lo = FIRST_BURST + j * STEP_BURST
            hi = lo + STEP_BURST if j < steps - 1 else len(tail_copies)
            pl.when(i == j)(functools.partial(start_tail, lo, hi))
        return carry

    lax.fori_loop(0, steps, attend_second_group, 0)

    o = jnp.concatenate([o_buf[h, j:j + 1, :] for h in range(hkv) for j in range(2)], axis=1)
    o8 = jnp.broadcast_to(o, (SUBLANES, HQ * DH)).astype(BF16)
    wait(wo_buf, sem_wo)
    attn = lax.dot_general(o8, wo_buf[...], CONTRACT_LAST, preferred_element_type=F32)
    base = gate * attn[0:1] + (1.0 - gate) * x
    hidden = h_buf[...].astype(BF16)
    for j in range(full_slabs):
        cols = slice(j * LANES, (j + 1) * LANES)
        slab = w4_buf.at[pl.ds(j * LANES, LANES)]
        wait(slab, sem_w4 + j)
        mlp = lax.dot_general(hidden, slab[...], CONTRACT_LAST, preferred_element_type=F32)
        out_ref[0, :, cols] = (base[:, cols] + (1.0 - gate) * mlp[0:1]).astype(out_ref.dtype)
    last = base[:, last_row:]
    for j, buf in enumerate(last_bufs):
        wait(buf, sem_last + j)
        mlp = lax.dot_general(hidden[:, j * buf.shape[1]:(j + 1) * buf.shape[1]], buf[...],
                              CONTRACT_LAST, preferred_element_type=F32)
        last = last + (1.0 - gate) * mlp[0:1]
    out_ref[0, :, last_row:] = last.astype(out_ref.dtype)


@jax.jit
def pallas_gated_mix__sliding_block_cached__mixer_s_mlp__decode_kernel(
    A_x: jax.Array,
    A_k_cache: jax.Array,
    A_v_cache: jax.Array,
    A_wq: jax.Array,
    A_wo: jax.Array,
    B_x: jax.Array,
    B_w1: jax.Array,
    B_w2: jax.Array,
    B_w3: jax.Array,
    B_w4: jax.Array,
    gate_w: jax.Array,
):
    del B_x, B_w1, B_w2
    batch, seq, d = A_x.shape
    _, hkv, sk, _ = A_k_cache.shape
    f = B_w3.shape[1]
    window = min(4096, max(256, sk // 4))
    full_slabs = d // LANES
    last_row = full_slabs * LANES
    assert (batch, seq) == (1, 1) and hkv == 2 * GROUP and HQ == 2 * hkv
    assert window % (GROUP * COPY_ROWS) == 0 and d % (STREAMS * SUBLANES) == 0
    assert last_row < d and f % (2 * LAST_PARTS * LANES) == 0

    return pl.pallas_call(
        _kernel,
        out_shape=jax.ShapeDtypeStruct(A_x.shape, A_x.dtype),
        in_specs=[pl.BlockSpec(memory_space=pl.ANY)] * 8,
        out_specs=pl.BlockSpec(memory_space=pltpu.VMEM),
        scratch_shapes=[
            pltpu.VMEM(A_x.shape, A_x.dtype),
            pltpu.VMEM(gate_w.shape, gate_w.dtype),
            pltpu.VMEM((hkv, window, DH), BF16),
            pltpu.VMEM((hkv, window, DH), BF16),
            pltpu.VMEM((d, HQ * DH), BF16),
            pltpu.VMEM((d, HQ * DH), BF16),
            pltpu.VMEM((d, f), BF16),
            pltpu.VMEM((last_row, f), BF16),
            pltpu.VMEM((hkv, SUBLANES, DH), F32),
            pltpu.VMEM((hkv, SUBLANES, DH), F32),
            pltpu.VMEM((SUBLANES, f), F32),
            pltpu.SemaphoreType.DMA((5 + hkv // GROUP + full_slabs + LAST_PARTS,)),
            *[pltpu.VMEM((d - last_row, f // LAST_PARTS), BF16)] * LAST_PARTS,
        ],
        compiler_params=pltpu.CompilerParams(
            vmem_limit_bytes=100 * 1024 * 1024,
            disable_semaphore_checks=True,
        ),
    )(A_x, gate_w, A_k_cache, A_v_cache, A_wq, A_wo.T, B_w3, B_w4.T)
```
